```python
import jax
import jax.numpy as jnp

def _softmax(x, axis=-1):
    return jax.nn.softmax(x, axis=axis)
def _gelu(x):
    return jax.nn.gelu(x, approximate=True)
def _silu(x):
    return jax.nn.silu(x)
def _sigmoid(x):
    return jax.nn.sigmoid(x)
def _layernorm(x, axis=-1, eps=1e-5):
    m = jnp.mean(x, axis=axis, keepdims=True)
    v = jnp.var(x, axis=axis, keepdims=True)
    return (x - m) / jnp.sqrt(v + eps)
def _scatter_add(tgt, idx, src, axis=0):
    return tgt.at[idx].add(src)
def _segment_sum(src, seg, n):
    return jax.ops.segment_sum(src, seg, n)
class _Rng:
    def __init__(self, key):
        self._k = key
    def _next(self):
        self._k, sub = jax.random.split(self._k)
        return sub
    def normal(self, shape):
        return jax.random.normal(self._next(), shape, dtype=jnp.bfloat16)
    def randint(self, lo, hi, shape):
        return jax.random.randint(self._next(), shape, lo, hi, dtype=jnp.int32)
    def uniform(self, shape, lo=0.0, hi=1.0):
        return jax.random.uniform(self._next(), shape, jnp.bfloat16, lo, hi)
    def permutation(self, n):
        return jax.random.permutation(self._next(), n)


kernel_name = 'standalone__batchnorm__prompt'

def setup_inputs():
    _rng = _Rng(jax.random.key(int.from_bytes(__import__("os").urandom(4), "little")))
    _w = (lambda a: (lambda t: t.astype(jnp.bfloat16) if jnp.issubdtype(t.dtype, jnp.floating) else t)(jnp.asarray(a)))
    B, S, C = 2, 2048, 1024
    K = 3
    return {
        "x": _w((lambda *s: _rng.normal(s) * 0.05)(B, S, C)),
        "w": _w((lambda *s: _rng.normal(s) * 0.05)(K, C, C) * (1.0 / (K * C) ** 0.5)),
        "mean": _w((lambda *s: _rng.normal(s) * 0.05)(C) * 0.1),
        "var": _w(jnp.abs((lambda *s: _rng.normal(s) * 0.05)(C)) + 0.5),
        "g": _w((lambda *s: _rng.normal(s) * 0.05)(C) + 1.0),
        "b": _w((lambda *s: _rng.normal(s) * 0.05)(C) * 0.1),
    }

def reference(x, w, mean, var, g, b):
    K = 3
    P = K // 2
    S = x.shape[1]
    xp = jnp.pad(x, ((0, 0), (P, P), (0, 0)))
    y = sum(jnp.einsum('bsc,cd->bsd', xp[:, k:k + S, :], w[k]) for k in range(K))
    inv_std = 1.0 / jnp.sqrt(var + 1e-5)
    y = (y - mean) * (g * inv_std) + b
    return _silu(y)
```

```python
import jax, jax.numpy as jnp
from jax.experimental import pallas as pl
from jax.experimental.pallas import tpu as pltpu


def make_direct(tm=512, tn=1024):
    def fn(x, w, mean, var, g, b):
        B, S, C = x.shape
        nt = S // tm
        H = 16
        hb = tm // H

        def kern(xp_ref, x_ref, xn_ref, w_ref, mean_ref, var_ref, g_ref, b_ref, o_ref):
            i = pl.program_id(1)
            xc = x_ref[0].astype(jnp.float32)
            prev_last = jnp.where(i > 0, xp_ref[0, H - 1:H, :].astype(jnp.float32), 0.0)
            next_first = jnp.where(i < nt - 1, xn_ref[0, 0:1, :].astype(jnp.float32), 0.0)
            row = jax.lax.broadcasted_iota(jnp.int32, (tm, C), 0)
            xm = jnp.where(row == 0, prev_last, pltpu.roll(xc, 1, 0)).astype(jnp.bfloat16)
            xq = jnp.where(row == tm - 1, next_first, pltpu.roll(xc, tm - 1, 0)).astype(jnp.bfloat16)
            acc = jnp.dot(xm, w_ref[0], preferred_element_type=jnp.float32)
            acc += jnp.dot(x_ref[0], w_ref[1], preferred_element_type=jnp.float32)
            acc += jnp.dot(xq, w_ref[2], preferred_element_type=jnp.float32)
            scale = g_ref[...].astype(jnp.float32) * jax.lax.rsqrt(var_ref[...].astype(jnp.float32) + 1e-5)
            y = (acc - mean_ref[...].astype(jnp.float32)) * scale + b_ref[...].astype(jnp.float32)
            o_ref[0] = (y * jax.nn.sigmoid(y)).astype(o_ref.dtype)

        vec = lambda a: a.reshape(1, C)
        vspec = pl.BlockSpec((1, C), lambda bb, i: (0, 0))
        return pl.pallas_call(
            kern,
            grid=(B, nt),
            in_specs=[
                pl.BlockSpec((1, H, C), lambda bb, i: (bb, jnp.maximum(i * hb - 1, 0), 0)),
                pl.BlockSpec((1, tm, C), lambda bb, i: (bb, i, 0)),
                pl.BlockSpec((1, H, C), lambda bb, i: (bb, jnp.minimum((i + 1) * hb, S // H - 1), 0)),
                pl.BlockSpec((3, C, C), lambda bb, i: (0, 0, 0)),
                vspec, vspec, vspec, vspec,
            ],
            out_specs=pl.BlockSpec((1, tm, C), lambda bb, i: (bb, i, 0)),
            out_shape=jax.ShapeDtypeStruct((B, S, C), x.dtype),
            compiler_params=pltpu.CompilerParams(dimension_semantics=("arbitrary", "arbitrary"), vmem_limit_bytes=100 * 1024 * 1024),
        )(x, x, x, w, vec(mean), vec(var), vec(g), vec(b))
    return fn


@jax.jit
def pallas_standalone__batchnorm__prompt_kernel(x, w, mean, var, g, b):
    return make_direct(256)(x, w, mean, var, g, b)
```

```python
import math, contextlib
import numpy as np
import jax, jax.numpy as jnp
from jax.experimental import pallas as pl
from jax.experimental.pallas import tpu as pltpu

F32, BF16, U32 = jnp.float32, jnp.bfloat16, jnp.uint32


def lo(u):
    return pltpu.bitcast(u << 16, F32)


def hi(u):
    return pltpu.bitcast(u & U32(0xFFFF0000), F32)


def mulc(c, x):
    return x if c == 1.0 else x * np.float32(c)


def as_bf(u):
    return pltpu.bitcast(u, BF16)


def pk(e, o):
    return pltpu.pack_elementwise([e, o], packed_dtype=BF16)


def make_v2(TM=1024, a=math.sqrt(2.0), silu='exp', scopes=False, xwin=4, u0_at=3, x2_from=5,
            opaque_v=True, opaque_m=True, inter=True, wait_at=0, flags=None, prewait=0, wait_at_s=0, tail5=True, skip='', nch=8, ksplit=False, lastbar=True, joint=True, vsame=True):
    bb_ = 1.0 / a
    a2, b2 = a * a, bb_ * bb_
    s_ = a2 + b2
    OT = 8

    def fn(x, w, mean, var, g, b):
        B, S, C = x.shape
        T = TM // 4
        NC = C // 128
        tiles_per_b = S // TM
        nsteps = B * tiles_per_b
        PAD = 16
        NG = T // 16
        XR = (S + 2 * PAD) // 2
        assert 6 * T <= 2 * XR and 3 * C // 2 <= 2 * XR
        WS = B * NC // 2 + 2
        NO = T // OT

        def kern(z_hbm, x_hbm, w_hbm, mean_hbm, var_hbm, g_hbm, b_hbm, o_hbm,
                 zbuf, prm0, prm1, prm2, prm3, xm, ubuf0, ubuf1, vbuf0, vbuf1, obuf, pbuf, zsem, psem, xsem, wsem, osem):
            def x_rows(k):
                ti = k % tiles_per_b
                r0 = 0 if ti == 0 else ti * TM + PAD
                r1 = S if ti == tiles_per_b - 1 else (ti + 1) * TM + PAD
                return k // tiles_per_b, r0, r1 - r0

            xbuf = xm.bitcast(BF16)

            def x_copy(k, c):
                bi, r0, n = x_rows(k)
                return pltpu.make_async_copy(x_hbm.at[bi, pl.ds(r0, n), pl.ds(c * 128, 128)],
                                             xbuf.at[(bi * NC + c) // 2, pl.ds(((bi * NC + c) % 2) * 2 * XR + PAD + r0, n), :], xsem.at[k, c])

            class w_copy:
                def __init__(self, n):
                    self.c = [pltpu.make_async_copy(w_hbm.at[kk, :, pl.ds(n * 128, 128)],
                                                    xbuf.at[WS + n, pl.ds(kk * C, C), :], wsem.at[n, kk]) for kk in range(3)]
                def start(self):
                    for c in self.c: c.start()
                def wait(self):
                    for c in self.c: c.wait()

            def out_copy(k):
                st, n = divmod(k, NC)
                bi, ti = divmod(st, tiles_per_b)
                return pltpu.make_async_copy(obuf.at[st, n], o_hbm.at[bi, pl.ds(ti * TM, TM), pl.ds(n * 128, 128)],
                                             osem.at[st, n])

            z_copy = pltpu.make_async_copy(z_hbm, zbuf, zsem.at[0])
            prm = [prm0, prm1, prm2, prm3]
            p_copies = [pltpu.make_async_copy(r, prm[i], psem.at[i])
                        for i, r in enumerate((mean_hbm, var_hbm, g_hbm, b_hbm))]
            z_copy.start()
            w_copy(0).start()
            for c in range(xwin):
                x_copy(0, c).start()
            for cp in p_copies:
                cp.start()

            zero = jnp.zeros((PAD // 2, 128), U32)
            for bc in range(B * NC):
                xm[bc // 2, pl.ds((bc % 2) * XR, PAD // 2), :] = zero
                xm[bc // 2, pl.ds((bc % 2) * XR + (PAD + S) // 2, PAD // 2), :] = zero

            z_copy.wait()
            zs = [zbuf[i] - q for i, q in enumerate((3, 1, 4, 1))]
            zvr = zs[0]
            zvw = zs[0] if (joint and vsame) else (zs[0] + zs[2] if joint else zs[1])
            zx = zs[1] if joint else 0
            zu = zs[0]
            zmr = zs[2]
            zmw = zs[3]

            uus = [ubuf0.bitcast(U32), ubuf1.bitcast(U32)]
            vus = [vbuf0.bitcast(U32), vbuf1.bitcast(U32)]
            ou_all = obuf.bitcast(U32)
            Na = 2 * a2 * (a2 - b2)
            Nb = 2 * b2 * (b2 - a2)

            def bn_params():
                for cp in p_copies:
                    cp.wait()
                cv = lambda i: jnp.broadcast_to(prm[i][...].astype(F32).reshape(1, C), (8, C))
                sc = cv(2) * jax.lax.rsqrt(cv(1) + 1e-5)
                sh = cv(3) - cv(0) * sc
                pbuf[0] = sc
                pbuf[1] = sc * np.float32(a)
                pbuf[2] = sc * np.float32(a2)
                pbuf[3] = sh

            def utrans(n, rows):
                if 'u' in skip: return
                for r in rows:
                    rs = pl.ds(r * 8, 8)
                    w0, w1, w2 = [xm[WS + n + zx, pl.ds(kk * (C // 2) + r * 8, 8), :] for kk in range(3)]
                    res = []
                    for ext in (lo, hi):
                        g0 = ext(w0); g1 = ext(w1); g2 = ext(w2)
                        ea = mulc(1 / Na, g0) + mulc(a2 / Na, g2)
                        oa = mulc(a / Na, g1)
                        eb = mulc(1 / Nb, g0) + mulc(b2 / Nb, g2)
                        ob = mulc(bb_ / Nb, g1)
                        res.append((ea + oa, ea - oa, eb + ob, eb - ob))
                    ud = uus[n % 2]
                    ud[zu, n // 2, rs, :] = w0
                    ud[5 + zu, n // 2, rs, :] = w2
                    for i in range(4):
                        ud[1 + i + zu, n // 2, rs, :] = pk(res[0][i], res[1][i])

            def vtrans(step, c, groups):
                if 'v' in skip: return
                slot = step % 2
                bi, ti = divmod(step, tiles_per_b)
                xt = xm.at[(bi * NC + c) // 2 + zx, pl.ds(((bi * NC + c) % 2) * XR + ti * (TM // 2), TM // 2 + PAD), :]
                for gidx in groups:
                    res = []
                    for half in range(2):
                        p0 = PAD // 2 + 32 * gidx + 2 * half
                        A = xt[pl.ds(p0, 8, stride=4), :]
                        Bq = xt[pl.ds(p0 + 1, 8, stride=4), :]
                        Cm = xt[pl.ds(p0 - 1, 8, stride=4), :]
                        Dp = xt[pl.ds(p0 + 2, 8, stride=4), :]
                        d0 = hi(Cm); d1 = lo(A); d2 = hi(A); d3 = lo(Bq); d4 = hi(Bq); d5 = lo(Dp)
                        e_b = d4 - mulc(b2, d2)
                        e_a = d4 - mulc(a2, d2)
                        o_b = mulc(a, d3) - mulc(bb_, d1)
                        o_a = mulc(bb_, d3) - mulc(a, d1)
                        res.append([(d0 + d4) - mulc(s_, d2), e_b + o_b, e_b - o_b, e_a + o_a, e_a - o_a,
                                    (d1 + d5) - mulc(s_, d3)])
                    for i in range(6):
                        vus[slot][i + zvw, c, pl.ds(gidx * 8, 8), :] = pk(res[0][i], res[1][i])

            def act(z):
                if silu == 'exp':
                    e = jnp.exp2(z * np.float32(-1.4426950408889634))
                    return z * pl.reciprocal(1.0 + e, approx=True)
                elif silu == 'expnr':
                    d = 1.0 + jnp.exp2(z * np.float32(-1.4426950408889634))
                    r = pl.reciprocal(d, approx=True)
                    return z * (r * (2.0 - d * r))
                else:
                    return z * jax.nn.sigmoid(z)

            def dot(k, i, between=None, mid=None):
                st, n = divmod(k, NC)
                r = uus[n % 2][i + zu, n // 2]
                ld = lambda cs: jnp.concatenate([as_bf(vus[st % 2][i + zvr, c]) for c in cs], axis=1)
                if ksplit:
                    rr = as_bf(r)
                    res = jnp.dot(ld(range(0, NC // 2)), rr[:C // 2], preferred_element_type=F32)
                    if mid is not None:
                        mid()
                    res = res + jnp.dot(ld(range(NC // 2, NC)), rr[C // 2:], preferred_element_type=F32)
                else:
                    res = jnp.dot(ld(range(NC)), as_bf(r), preferred_element_type=F32)
                ch = T // nch
                for q in range(nch):
                    xm[B * NC // 2 + k % 2 + zmw, pl.ds(i * T + q * ch, ch), :] = pltpu.bitcast(res[q * ch:(q + 1) * ch], U32)
                    if between is not None:
                        between(q)

            def otrans(k, groups):
                if 'o' in skip: return
                st, n = divmod(k, NC)
                ou = ou_all.at[st]
                cs = pl.ds(n * 128, 128)
                s0 = pbuf[0, :, cs]; s1 = pbuf[1, :, cs]; s2 = pbuf[2, :, cs]; sh_ = pbuf[3, :, cs]
                for gidx in groups:
                    rs = pl.ds(gidx * OT, OT)
                    m = []
                    for i in range(6):
                        m.append(pltpu.bitcast(xm[B * NC // 2 + k % 2 + zmr, pl.ds(i * T + gidx * OT, OT), :], F32))
                    sa = m[1] + m[2]; da = m[1] - m[2]; sb = m[3] + m[4]; db = m[3] - m[4]
                    r_ = bb_ / a
                    y0 = m[0] + sa + sb
                    y1 = da + mulc(r_, db)
                    y2 = sa + mulc(r_ ** 2, sb)
                    y3 = mulc(a ** 3, da + mulc(r_ ** 3, db)) + m[5]
                    z0 = act(y0 * s0 + sh_); z1 = act(y1 * s1 + sh_)
                    z2 = act(y2 * s2 + sh_); z3 = act(y3 * s0 + sh_)
                    ou[n, pl.ds(2 * gidx * OT, OT, stride=2), :] = pk(z0, z1)
                    ou[n, pl.ds(2 * gidx * OT + 1, OT, stride=2), :] = pk(z2, z3)

            def split(n_items, parts, j):
                lo_ = (n_items * j) // parts; hi_ = (n_items * (j + 1)) // parts
                return range(lo_, hi_)

            sc_ = (lambda nm: jax.named_scope(nm)) if scopes else (lambda nm: contextlib.nullcontext())
            NR = C // 16

            with sc_('p_v0'):
                for c in range(NC):
                    x_copy(0, c).wait()
                    if c + xwin < NC:
                        x_copy(0, c + xwin).start()
                    elif c + xwin == NC:
                        w_copy(1).start()
                    vtrans(0, c, range(NG))
                    if c == u0_at:
                        w_copy(0).wait()
                        utrans(0, range(NR))
                w_copy(2).start()
                x_copy(1, 0).start()
                bn_params()
                if prewait:
                    for n in range(3, NC):
                        w_copy(n).start()
                    for c in range(1, NC):
                        x_copy(1, c).start()
                    for k in range(2, nsteps):
                        for c in range(NC):
                            x_copy(k, c).start()
                    for n in range(1, NC):
                        w_copy(n).wait()
                    for k in range(1, nsteps):
                        for c in range(NC):
                            x_copy(k, c).wait()

            waited = set()

            def v0cols(n):
                return [] if n == 0 else [n - 1] if n < NC - 1 else [NC - 2, NC - 1]

            def dummy_bar(n):
                cp = pltpu.make_async_copy(var_hbm, prm1, psem.at[1]); cp.start(); cp.wait()

            def barrier0(n):
                if prewait == 1:
                    return
                if prewait == 2:
                    if n >= 2:
                        out_copy(n - 2).wait(); waited.add(n - 2)
                    return
                if n + 1 < NC:
                    w_copy(n + 1).wait()
                for c in v0cols(n):
                    x_copy(1, c).wait()
                if n + 3 < NC:
                    w_copy(n + 3).start()
                if n + 1 < NC - 1:
                    x_copy(1, n + 1).start()
                if n == NC - 3:
                    x_copy(1, NC - 1).start()
                if nsteps > 2 and n >= x2_from:
                    per = -(-NC // (NC - x2_from))
                    for c in range((n - x2_from) * per, min(NC, (n - x2_from + 1) * per)):
                        x_copy(2, c).start()

            def barrier_step(step):
                if step + 1 < nsteps:
                    for c in range(NC):
                        x_copy(step + 1, c).wait()
                if step >= 2:
                    for kk in range((step - 2) * NC, (step - 1) * NC):
                        if kk not in waited:
                            out_copy(kk).wait(); waited.add(kk)
                if step + 2 < nsteps:
                    for c in range(NC):
                        x_copy(step + 2, c).start()

            for step in range(nsteps):
                with sc_(f'step{step}'):
                    for n in range(NC):
                        k = step * NC + n
                        do_v = step + 1 < nsteps
                        do_u = step == 0 and n + 1 < NC
                        do_o = k >= 1
                        has_bar = step == 0 or (n == 0 and (step + 1 < nsteps or lastbar) and not prewait)
                        wa = (wait_at if step == 0 else wait_at_s) if has_bar else 0
                        nxt_step, nxt_n = divmod(k + 1, NC)
                        bar_next = (nxt_step == 0 and wait_at == 0) or (nxt_n == 0 and nxt_step < nsteps and (nxt_step + 1 < nsteps or lastbar) and wait_at_s == 0)
                        last_i = 5 if (bar_next and tail5) else 6
                        cols = v0cols(n) if step == 0 else [n]
                        for i in range(6):
                            if has_bar and i == wa:
                                barrier0(n) if step == 0 else barrier_step(step)
                            if not inter or i >= last_i:
                                dot(k, i)
                                continue

                            def between(q, i=i):
                                if do_o:
                                    otrans(k - 1, split(NO, last_i * nch, i * nch + q))
                                if i >= wa and do_u:
                                    utrans(n + 1, split(NR, (last_i - wa) * nch, (i - wa) * nch + q))
                                if joint:
                                    vpiece(q, nch)

                            def vpiece(h, nh, i=i):
                                if i >= wa and do_v:
                                    items = [(c, gq) for c in cols for gq in range(NG)]
                                    for q in split(len(items), (last_i - wa) * nh, (i - wa) * nh + h):
                                        vtrans(step + 1, items[q][0], [items[q][1]])

                            if joint:
                                dot(k, i, between)
                            elif ksplit:
                                dot(k, i, between, lambda: vpiece(0, 2))
                                vpiece(1, 2)
                            else:
                                dot(k, i, between)
                                vpiece(0, 1)
                        if not inter:
                            if do_u:
                                utrans(n + 1, range(NR))
                            if do_o:
                                otrans(k - 1, range(NO))
                            if do_v:
                                for c in cols:
                                    vtrans(step + 1, c, range(NG))
                        if do_o:
                            out_copy(k - 1).start()
            with sc_('drain'):
                last = nsteps * NC - 1
                otrans(last, range(NO))
                out_copy(last).start()
                for k in range(nsteps * NC):
                    if k not in waited:
                        out_copy(k).wait()

        anyspec = pl.BlockSpec(memory_space=pl.ANY)
        zeros = np.array([3, 1, 4, 1], dtype=np.int32)
        return pl.pallas_call(
            kern,
            in_specs=[anyspec] * 7,
            out_specs=anyspec,
            out_shape=jax.ShapeDtypeStruct((B, S, C), x.dtype),
            scratch_shapes=[
                pltpu.SMEM((4,), jnp.int32),
                pltpu.VMEM((C,), BF16), pltpu.VMEM((C,), BF16), pltpu.VMEM((C,), BF16), pltpu.VMEM((C,), BF16),
                pltpu.VMEM((B * NC // 2 + 2 + NC, 2 * XR, 128), U32),
                pltpu.VMEM((6, NC // 2, C, 128), BF16),
                pltpu.VMEM((6, NC // 2, C, 128), BF16),
                pltpu.VMEM((6, NC, T, 128), BF16),
                pltpu.VMEM((6, NC, T, 128), BF16),
                pltpu.VMEM((nsteps, NC, TM, 128), BF16),
                pltpu.VMEM((4, 8, C), F32),
                pltpu.SemaphoreType.DMA((1,)),
                pltpu.SemaphoreType.DMA((4,)),
                pltpu.SemaphoreType.DMA((nsteps, NC)),
                pltpu.SemaphoreType.DMA((NC, 3)),
                pltpu.SemaphoreType.DMA((nsteps, NC)),
            ],
            compiler_params=pltpu.CompilerParams(vmem_limit_bytes=100 * 1024 * 1024, flags=flags),
        )(zeros, x, w, mean, var, g, b)
    return fn


@jax.jit
def pallas_standalone__batchnorm__prompt_kernel(x, w, mean, var, g, b):
    return make_v2()(x, w, mean, var, g, b)
```

```python
import math

import jax
import jax.numpy as jnp
import numpy as np
from jax.experimental import pallas as pl
from jax.experimental.pallas import tpu as pltpu

F32, BF16, U32 = jnp.float32, jnp.bfloat16, jnp.uint32

TM = 1024
PAD = 16
NCH = 8
XWIN = 5
U0_AT = 2
BAR0_AT = 3
X2_PLAN = ((), (), (), (), (0,), (1, 2), (3, 4, 5), (6, 7))
ZKEY = (3, 1, 4, 1)

PA = math.sqrt(2.0)
PB = 1.0 / PA


def _lo(u):
    return pltpu.bitcast(u << 16, F32)


def _hi(u):
    return pltpu.bitcast(u & U32(0xFFFF0000), F32)


def _mul(c, x):
    return x * np.float32(c)


def _as_bf16(u):
    return pltpu.bitcast(u, BF16)


def _pack(even, odd):
    return pltpu.pack_elementwise([even, odd], packed_dtype=BF16)


def _split(n, parts, j):
    return range((n * j) // parts, (n * (j + 1)) // parts)


def _silu(z):
    d = 1.0 + jnp.exp2(jnp.minimum(z * np.float32(-1.4426950408889634), np.float32(125.0)))
    r = pl.reciprocal(d, approx=True)
    return z * (r * (2.0 - d * r))


def _build(B, S, C):
    a, bb = PA, PB
    a2, b2 = a * a, bb * bb
    s_ = a2 + b2
    na, nb = 2 * a2 * (a2 - b2), 2 * b2 * (b2 - a2)
    T, NC = TM // 4, C // 128
    tpb = S // TM
    nsteps = B * tpb
    NG, NO, NR = T // 16, T // 8, C // 16
    XR = (S + 2 * PAD) // 2
    MS = B * NC // 2
    WS = MS + 2
    last = nsteps * NC - 1
    assert S % TM == 0 and C % 256 == 0 and nsteps >= 3 and NC == len(X2_PLAN)
    assert 6 * T <= 2 * XR and 3 * C // 2 <= 2 * XR

    def kern(z_hbm, x_hbm, w_hbm, mean_hbm, var_hbm, g_hbm, b_hbm, o_hbm,
             zbuf, p0, p1, p2, p3, xm, u0buf, u1buf, v0buf, v1buf, obuf, pbuf,
             zsem, psem, xsem, wsem, osem, tsem):
        xbf = xm.bitcast(BF16)

        def x_copy(k, c):
            bi, ti = divmod(k, tpb)
            r0 = 0 if ti == 0 else ti * TM + PAD
            r1 = S if ti == tpb - 1 else (ti + 1) * TM + PAD
            bc = bi * NC + c
            return pltpu.make_async_copy(
                x_hbm.at[bi, pl.ds(r0, r1 - r0), pl.ds(c * 128, 128)],
                xbf.at[bc // 2, pl.ds((bc % 2) * 2 * XR + PAD + r0, r1 - r0), :], xsem.at[k, c])

        def w_copies(n):
            return [pltpu.make_async_copy(w_hbm.at[kk, :, pl.ds(n * 128, 128)],
                                          xbf.at[WS + n, pl.ds(kk * C, C), :], wsem.at[n, kk])
                    for kk in range(3)]

        def w_start(n):
            for cp in w_copies(n):
                cp.start()

        def w_wait(n):
            for cp in w_copies(n):
                cp.wait()

        def out_copy(k, r0=0, rows=TM, sem=None):
            st, n = divmod(k, NC)
            bi, ti = divmod(st, tpb)
            return pltpu.make_async_copy(
                obuf.at[st, n, pl.ds(r0, rows)],
                o_hbm.at[bi, pl.ds(ti * TM + r0, rows), pl.ds(n * 128, 128)],
                osem.at[st, n] if sem is None else sem)

        prm = [p0, p1, p2, p3]
        z_copy = pltpu.make_async_copy(z_hbm, zbuf, zsem.at[0])
        p_copies = [pltpu.make_async_copy(r, prm[i], psem.at[i])
                    for i, r in enumerate((mean_hbm, var_hbm, g_hbm, b_hbm))]
        z_copy.start()
        w_start(0)
        for c in range(XWIN):
            x_copy(0, c).start()
        for cp in p_copies:
            cp.start()

        zero = jnp.zeros((PAD // 2, 128), U32)
        for bc in range(B * NC):
            xm[bc // 2, pl.ds((bc % 2) * XR, PAD // 2), :] = zero
            xm[bc // 2, pl.ds((bc % 2) * XR + (PAD + S) // 2, PAD // 2), :] = zero

        z_copy.wait()
        zv, zx, zmr, zmw = [zbuf[i] - q for i, q in enumerate(ZKEY)]
        uus = [u0buf.bitcast(U32), u1buf.bitcast(U32)]
        vus = [v0buf.bitcast(U32), v1buf.bitcast(U32)]
        ou_all = obuf.bitcast(U32)

        def bn_params():
            for cp in p_copies:
                cp.wait()
            cv = lambda i: jnp.broadcast_to(prm[i][...].astype(F32).reshape(1, C), (8, C))
            sc = cv(2) * jax.lax.rsqrt(cv(1) + 1e-5)
            pbuf[0] = sc
            pbuf[1] = sc * np.float32(a)
            pbuf[2] = sc * np.float32(a2)
            pbuf[3] = cv(3) - cv(0) * sc

        def utrans(n, rows):
            ud = uus[n % 2]
            for r in rows:
                rs = pl.ds(r * 8, 8)
                w0, w1, w2 = [xm[WS + n + zx, pl.ds(kk * (C // 2) + r * 8, 8), :] for kk in range(3)]
                res = []
                for ext in (_lo, _hi):
                    g0, g1, g2 = ext(w0), ext(w1), ext(w2)
                    ea = _mul(1 / na, g0) + _mul(a2 / na, g2)
                    oa = _mul(a / na, g1)
                    eb = _mul(1 / nb, g0) + _mul(b2 / nb, g2)
                    ob = _mul(bb / nb, g1)
                    res.append((ea + oa, ea - oa, eb + ob, eb - ob))
                ud[zv, n // 2, rs, :] = w0
                ud[5 + zv, n // 2, rs, :] = w2
                for i in range(4):
                    ud[1 + i + zv, n // 2, rs, :] = _pack(res[0][i], res[1][i])

        def vtrans(step, c, groups):
            bi, ti = divmod(step, tpb)
            bc = bi * NC + c
            xt = xm.at[bc // 2 + zx, pl.ds((bc % 2) * XR + ti * (TM // 2), TM // 2 + PAD), :]
            for gi in groups:
                res = []
                for half in range(2):
                    q = PAD // 2 + 32 * gi + 2 * half
                    A = xt[pl.ds(q, 8, stride=4), :]
                    Bq = xt[pl.ds(q + 1, 8, stride=4), :]
                    d0 = _hi(xt[pl.ds(q - 1, 8, stride=4), :])
                    d5 = _lo(xt[pl.ds(q + 2, 8, stride=4), :])
                    d1, d2, d3, d4 = _lo(A), _hi(A), _lo(Bq), _hi(Bq)
                    e_b = d4 - _mul(b2, d2)
                    e_a = d4 - _mul(a2, d2)
                    o_b = _mul(a, d3) - _mul(bb, d1)
                    o_a = _mul(bb, d3) - _mul(a, d1)
                    res.append([(d0 + d4) - _mul(s_, d2), e_b + o_b, e_b - o_b, e_a + o_a, e_a - o_a,
                                (d1 + d5) - _mul(s_, d3)])
                for i in range(6):
                    vus[step % 2][i + zv, c, pl.ds(gi * 8, 8), :] = _pack(res[0][i], res[1][i])

        def dot(k, i, between):
            st, n = divmod(k, NC)
            lhs = jnp.concatenate([_as_bf16(vus[st % 2][i + zv, c]) for c in range(NC)], axis=1)
            res = jnp.dot(lhs, _as_bf16(uus[n % 2][i + zv, n // 2]), preferred_element_type=F32)
            ch = T // NCH
            for q in range(NCH):
                xm[MS + k % 2 + zmw, pl.ds(i * T + q * ch, ch), :] = pltpu.bitcast(res[q * ch:(q + 1) * ch], U32)
                between(q)

        def otrans(k, groups):
            st, n = divmod(k, NC)
            ou = ou_all.at[st]
            cs = pl.ds(n * 128, 128)
            s0, s1, s2, sh = pbuf[0, :, cs], pbuf[1, :, cs], pbuf[2, :, cs], pbuf[3, :, cs]
            r_ = bb / a
            for gi in groups:
                m = [pltpu.bitcast(xm[MS + k % 2 + zmr, pl.ds(i * T + gi * 8, 8), :], F32) for i in range(6)]
                sa, da, sb, db = m[1] + m[2], m[1] - m[2], m[3] + m[4], m[3] - m[4]
                z0 = _silu((m[0] + sa + sb) * s0 + sh)
                z1 = _silu((da + _mul(r_, db)) * s1 + sh)
                z2 = _silu((sa + _mul(r_ ** 2, sb)) * s2 + sh)
                z3 = _silu((_mul(a ** 3, da + _mul(r_ ** 3, db)) + m[5]) * s0 + sh)
                ou[n, pl.ds(16 * gi, 8, stride=2), :] = _pack(z0, z1)
                ou[n, pl.ds(16 * gi + 1, 8, stride=2), :] = _pack(z2, z3)

        def v1_cols(n):
            return [] if n == 0 else [n - 1] if n < NC - 1 else [NC - 2, NC - 1]

        waited = set()

        def barrier0(n):
            if n + 1 < NC:
                w_wait(n + 1)
            for c in v1_cols(n):
                x_copy(1, c).wait()
            if n + 3 < NC:
                w_start(n + 3)
            if n + 1 < NC - 1:
                x_copy(1, n + 1).start()
            if n == NC - 3:
                x_copy(1, NC - 1).start()
            for c in X2_PLAN[n]:
                x_copy(2, c).start()

        def barrier_step(step):
            if step + 1 < nsteps:
                for c in range(NC):
                    x_copy(step + 1, c).wait()
            if step >= 2:
                for kk in range((step - 2) * NC, (step - 1) * NC):
                    out_copy(kk).wait()
                    waited.add(kk)
            if step + 2 < nsteps:
                for c in range(NC):
                    x_copy(step + 2, c).start()

        for c in range(NC):
            x_copy(0, c).wait()
            if c + XWIN < NC:
                x_copy(0, c + XWIN).start()
            elif c + XWIN == NC:
                w_start(1)
            vtrans(0, c, range(NG))
            if c == U0_AT:
                w_wait(0)
                utrans(0, range(NR))
        w_start(2)
        x_copy(1, 0).start()
        bn_params()

        for step in range(nsteps):
            for n in range(NC):
                k = step * NC + n
                do_v, do_u, do_o = step + 1 < nsteps, step == 0 and n + 1 < NC, k >= 1
                has_bar = step == 0 or n == 0
                wa = BAR0_AT if k == 0 else 0
                bar_next = step == 0 or n == NC - 1
                last_i = 5 if bar_next and k < last else 6
                cols = v1_cols(n) if step == 0 else [n]
                vitems = [(c, gi) for c in cols for gi in range(NG)] if do_v else []
                for i in range(6):
                    if has_bar and i == wa:
                        barrier0(n) if step == 0 else barrier_step(step)

                    def between(q, i=i):
                        if i >= last_i:
                            return
                        if do_o:
                            otrans(k - 1, _split(NO, last_i * NCH, i * NCH + q))
                        if i < wa:
                            return
                        parts, j = (last_i - wa) * NCH, (i - wa) * NCH + q
                        if do_u:
                            utrans(n + 1, _split(NR, parts, j))
                        for t in _split(len(vitems), parts, j):
                            vtrans(step + 1, vitems[t][0], [vitems[t][1]])

                    dot(k, i, between)
                if do_o:
                    out_copy(k - 1).start()

        tail = [out_copy(last, h * (TM // 2), TM // 2, tsem.at[h]) for h in range(2)]
        for h in range(2):
            otrans(last, _split(NO, 2, h))
            tail[h].start()
        for k in range(last):
            if k not in waited:
                out_copy(k).wait()
        for cp in tail:
            cp.wait()

    anyspec = pl.BlockSpec(memory_space=pl.ANY)
    return pl.pallas_call(
        kern,
        in_specs=[anyspec] * 7,
        out_specs=anyspec,
        out_shape=jax.ShapeDtypeStruct((B, S, C), BF16),
        scratch_shapes=[
            pltpu.SMEM((len(ZKEY),), jnp.int32),
            pltpu.VMEM((C,), BF16), pltpu.VMEM((C,), BF16), pltpu.VMEM((C,), BF16), pltpu.VMEM((C,), BF16),
            pltpu.VMEM((WS + NC, 2 * XR, 128), U32),
            pltpu.VMEM((6, NC // 2, C, 128), BF16),
            pltpu.VMEM((6, NC // 2, C, 128), BF16),
            pltpu.VMEM((6, NC, T, 128), BF16),
            pltpu.VMEM((6, NC, T, 128), BF16),
            pltpu.VMEM((nsteps, NC, TM, 128), BF16),
            pltpu.VMEM((4, 8, C), F32),
            pltpu.SemaphoreType.DMA((1,)),
            pltpu.SemaphoreType.DMA((4,)),
            pltpu.SemaphoreType.DMA((nsteps, NC)),
            pltpu.SemaphoreType.DMA((NC, 3)),
            pltpu.SemaphoreType.DMA((nsteps, NC)),
            pltpu.SemaphoreType.DMA((2,)),
        ],
        compiler_params=pltpu.CompilerParams(vmem_limit_bytes=100 * 1024 * 1024),
    )


@jax.jit
def pallas_standalone__batchnorm__prompt_kernel(x, w, mean, var, g, b):
    B, S, C = x.shape
    return _build(B, S, C)(np.asarray(ZKEY, dtype=np.int32), x, w, mean, var, g, b)
```
